```python
import os as _os
_os.environ.setdefault("JAX_PLATFORMS", "cpu")
import jax
import jax.numpy as jnp

def _softmax(x, axis=-1):
    return jax.nn.softmax(x, axis=axis)
def _gelu(x):
    return jax.nn.gelu(x, approximate=True)
def _silu(x):
    return jax.nn.silu(x)
def _sigmoid(x):
    return jax.nn.sigmoid(x)
def _layernorm(x, axis=-1, eps=1e-5):
    m = jnp.mean(x, axis=axis, keepdims=True)
    v = jnp.var(x, axis=axis, keepdims=True)
    return (x - m) / jnp.sqrt(v + eps)
def _scatter_add(tgt, idx, src, axis=0):
    return tgt.at[idx].add(src)
def _segment_sum(src, seg, n):
    return jax.ops.segment_sum(src, seg, n)
class _Rng:
    def __init__(self, key):
        self._k = key
    def _next(self):
        self._k, sub = jax.random.split(self._k)
        return sub
    def normal(self, shape):
        return jax.random.normal(self._next(), shape, dtype=jnp.bfloat16)
    def randint(self, lo, hi, shape):
        return jax.random.randint(self._next(), shape, lo, hi, dtype=jnp.int32)
    def uniform(self, shape, lo=0.0, hi=1.0):
        return jax.random.uniform(self._next(), shape, jnp.bfloat16, lo, hi)
    def permutation(self, n):
        return jax.random.permutation(self._next(), n)


kernel_name = 'sequential_preLN__sliding_block_cached__mixer_channel_mlp__decode'

def setup_inputs():
    _rng = _Rng(jax.random.key(int.from_bytes(__import__("os").urandom(4), "little")))
    _w = (lambda a: (lambda t: t.astype(jnp.bfloat16) if jnp.issubdtype(t.dtype, jnp.floating) else t)(jnp.asarray(a)))
    def _A_setup():
        B, Sq, D = 1, 1, 512
        Hq, Hkv, Sk, Dh = 32, 8, 65536, 128
        assert Hq % Hkv == 0, (Hq, Hkv)
        return {
            "x": _w((lambda *s: _rng.normal(s) * 0.05)(B, Sq, D)),
            "k_cache": _w((lambda *s: _rng.normal(s) * 3.2)(B, Hkv, Sk, Dh)),
            "v_cache": _w((lambda *s: _rng.normal(s) * 0.2)(B, Hkv, Sk, Dh)),
            "wq": _w((lambda *s: _rng.normal(s) * 3.2)(D, Hq * Dh) * (D ** -0.5)),
            "wo": _w((lambda *s: _rng.normal(s) * 0.2)(Hq * Dh, D) * ((Hq * Dh) ** -0.5)),
        }
    _A_in = _A_setup()

    def _B_setup():
        B, S, D, F = 1, 1, 512, 1792
        return {
            "x": _w((lambda *s: _rng.normal(s) * 0.05)(B, S, D)),
            "w1": _w((lambda *s: _rng.normal(s) * 0.2)(D, F) * (D ** -0.5)),
            "b1": _w((lambda *s: _rng.normal(s) * 0.2)(F)),
            "w2": _w((lambda *s: _rng.normal(s) * 0.2)(F, D) * (F ** -0.5)),
            "b2": _w((lambda *s: _rng.normal(s) * 0.05)(D)),
        }
    _B_in = _B_setup()

    return {
        "A_x": _A_in["x"],
        "A_k_cache": _A_in["k_cache"],
        "A_v_cache": _A_in["v_cache"],
        "A_wq": _A_in["wq"],
        "A_wo": _A_in["wo"],
        "B_x": _B_in["x"],
        "B_w1": _B_in["w1"],
        "B_b1": _B_in["b1"],
        "B_w2": _B_in["w2"],
        "B_b2": _B_in["b2"],
    }

def reference(A_x, A_k_cache, A_v_cache, A_wq, A_wo, B_x, B_w1, B_b1, B_w2, B_b2):
    def _A_ref(x, k_cache, v_cache, wq, wo):
        B, Sq, D = x.shape
        Hq, Dh = 32, 128
        Hkv, Sk = k_cache.shape[1], k_cache.shape[2]
        W = min(4096, max(256, Sk // 4))
        rep = Hq // Hkv
        q = (lambda x, *d: x.transpose(*d))((x @ wq).reshape(B, Sq, Hq, Dh), 0, 2, 1, 3)
        k = jnp.repeat(k_cache[:, :, Sk - W:, :], rep, axis=1)
        v = jnp.repeat(v_cache[:, :, Sk - W:, :], rep, axis=1)
        scores = jnp.einsum("bhqd,bhkd->bhqk", q, k) * (Dh ** -0.5)
        p = _softmax(scores, axis=-1)
        o = jnp.einsum("bhqk,bhkd->bhqd", p, v)
        return (lambda x, *d: x.transpose(*d))(o, 0, 2, 1, 3).reshape(B, Sq, Hq * Dh) @ wo

    def _B_ref(x, w1, b1, w2, b2):
        y = _layernorm(x, axis=-1)
        h = _gelu(jnp.einsum("bsd,df->bsf", y, w1) + b1)
        return jnp.einsum("bsf,fd->bsd", h, w2) + b2

    x = A_x
    h = x + _A_ref(_layernorm(x, axis=-1), A_k_cache, A_v_cache, A_wq, A_wo)
    h2 = h + _B_ref(_layernorm(h, axis=-1), B_w1, B_b1, B_w2, B_b2)
    return h2
```

```python
import jax
import jax.numpy as jnp
import numpy as np
from jax import lax
import jax.experimental.pallas as pl
import jax.experimental.pallas.tpu as pltpu

_F32 = jnp.float32
_EPS = 1e-5
_LANES = 128
_ROWS = 8

_PIECE = 16
_BLOCK = 32
_STRIDE = 8
_FIRST_BLOCK = {"w2": 24}
_FIRST_BLOCK_DEFAULT = 16
_LEAD = 27
_TAIL_PIECES = 3
_TAIL_TILES = 2
_AHEAD = 80
_STEP = 16
_W2_GROUPS = (16, 8, 8, 4, 2, 1, 1)


def _rects(shape, lo, hi):
    per_row = shape[1] // _LANES
    out = []
    while lo < hi:
        r, c = divmod(lo, per_row)
        if c == 0 and hi - lo >= per_row:
            n = (hi - lo) // per_row
            out.append((r * _ROWS, n * _ROWS, 0, shape[1]))
            lo += n * per_row
        else:
            n = min(per_row - c, hi - lo)
            out.append((r * _ROWS, _ROWS, c * _LANES, n * _LANES))
            lo += n
    return out


def _walk(names, shapes):
    blocks, whole = [], []
    for name in names:
        tiles = shapes[name][0] // _ROWS * (shapes[name][1] // _LANES)
        first = _FIRST_BLOCK.get(name, _FIRST_BLOCK_DEFAULT)
        starts = range(first, tiles - _BLOCK + 1, _BLOCK)
        whole.append([(name, lo, lo + _BLOCK) for lo in starts])
        edges = [(name, 0, first), (name, starts[-1] + _BLOCK, tiles)]
        blocks += [e for e in edges if e[2] > e[1]]
    for j in range(_STRIDE):
        for w in whole:
            blocks += w[j::_STRIDE]

    def halves(block):
        name, lo, hi = block
        return [(name, lo, hi - _PIECE), (name, hi - _PIECE, hi)] if hi - lo > _PIECE else [block]

    pieces = []
    for i in range(0, len(blocks), 2):
        pair = [halves(b) for b in blocks[i:i + 2]]
        for t in range(2):
            pieces += [p[t] for p in pair if t < len(p)]
    return pieces


def _plan(phases, shapes):
    pieces = [p for names in phases for p in _walk(names, shapes)]
    w2_group = [g + 1 for g, n in enumerate(_W2_GROUPS) for _ in range(n)]
    w2_group = [0] * (len(pieces) - len(w2_group)) + w2_group
    run = []
    for i, (name, lo, hi) in enumerate(pieces):
        group = ("w2", w2_group[i]) if name == "w2" else name
        if i < len(pieces) - _TAIL_PIECES:
            run += [(name, r, group, 1 - i % 2) for r in _rects(shapes[name], lo, hi)]
        else:
            for t in range(lo, hi, _TAIL_TILES):
                run += [(name, r, group, 1) for r in _rects(shapes[name], t, t + _TAIL_TILES)]
    low = [c for c in run if c[3] == 1]
    issue, rest = low[:_LEAD], low[_LEAD:][::-1]
    for c in run:
        if c[3] == 0:
            issue.append(c)
        elif rest:
            issue.append(rest.pop())
    return run, issue


@jax.jit
def pallas_sequential_preLN__sliding_block_cached__mixer_channel_mlp__decode_kernel(
    A_x: jax.Array,
    A_k_cache: jax.Array,
    A_v_cache: jax.Array,
    A_wq: jax.Array,
    A_wo: jax.Array,
    B_x: jax.Array,
    B_w1: jax.Array,
    B_b1: jax.Array,
    B_w2: jax.Array,
    B_b2: jax.Array,
):
    del B_x
    dtype = A_x.dtype
    d_model, d_ff = B_w1.shape
    _, n_kv, seq, d_head = A_k_cache.shape
    rep = A_wq.shape[1] // d_head // n_kv
    window = min(4096, max(256, seq // 4))
    assert A_x.shape == (1, 1, d_model) and d_head == _LANES and _ROWS % rep == 0
    scale = float(np.float32(d_head ** -0.5).astype(dtype))

    k_names = [("k", g) for g in range(n_kv)]
    v_names = [("v", g) for g in range(n_kv)]
    shapes = {"wq": A_wq.shape, "wo": A_wo.shape, "w1": B_w1.shape, "w2": B_w2.shape}
    shapes.update({name: (window, d_head) for name in k_names + v_names})
    run, issue = _plan((["wq"], k_names, v_names, ["wo"], ["w1"], ["w2"]), shapes)
    sem_of, due = {}, {}
    for n, c in enumerate(run):
        sem_of.setdefault(c[2], len(sem_of))
        due[c[2]] = n + _AHEAD
    for n, c in enumerate(issue):
        due[c[2]] = max(due[c[2]], n + 1)

    def rnd(a):
        return a.astype(dtype).astype(_F32)

    def layernorm(a):
        mean = jnp.mean(a, axis=-1, keepdims=True)
        var = jnp.mean(jnp.square(a - mean), axis=-1, keepdims=True)
        return rnd(rnd(a - rnd(mean)) / rnd(jnp.sqrt(rnd(rnd(var) + _EPS))))

    def kernel(x_hbm, k_hbm, v_hbm, wq_hbm, wo_hbm, w1_hbm, b1_hbm, w2_hbm, b2_hbm, out_hbm,
               x_ref, k_ref, v_ref, wq_ref, wo_ref, w1_ref, b1_ref, w2_ref, b2_ref, out_ref,
               p_ref, act_ref, sems, io_sem):
        refs = {"k": (k_hbm, k_ref), "v": (v_hbm, v_ref), "wq": (wq_hbm, wq_ref),
                "wo": (wo_hbm, wo_ref), "w1": (w1_hbm, w1_ref), "w2": (w2_hbm, w2_ref)}

        def copy(c):
            name, (row, rows, col, cols), group, _ = c
            if isinstance(name, tuple):
                src, dst = refs[name[0]]
                src = src.at[0, name[1], pl.ds(seq - window + row, rows), :]
                dst = dst.at[name[1], pl.ds(row, rows), :]
            else:
                src, dst = (r.at[pl.ds(row, rows), pl.ds(col, cols)] for r in refs[name])
            return pltpu.make_async_copy(src, dst, sems.at[sem_of[group]])

        started = 0

        def start_until(n):
            nonlocal started
            for c in issue[started:n]:
                copy(c).start(priority=c[3])
            started = max(started, min(n, len(issue)))

        def wait_for(group, buf):
            start_until(due[group])
            pltpu.make_async_copy(buf, buf, sems.at[sem_of[group]]).wait()

        start_until(_LEAD)
        vectors = [pltpu.make_async_copy(src, dst, io_sem)
                   for src, dst in ((x_hbm, x_ref), (b1_hbm, b1_ref), (b2_hbm, b2_ref))]
        for c in vectors:
            c.start()
        start_until(_LEAD + _AHEAD)
        for c in vectors:
            c.wait()

        x = jnp.broadcast_to(x_ref[0].astype(_F32), (_ROWS, d_model))
        xn = layernorm(x).astype(dtype)
        row_id = lax.broadcasted_iota(jnp.int32, (_ROWS, _LANES), 0)

        wait_for("wq", wq_ref)
        qs = []
        for g in range(n_kv):
            q = jnp.dot(xn, wq_ref[:, pl.ds(g * rep * d_head, rep * d_head)],
                        preferred_element_type=_F32)
            q_g = q[:, :d_head]
            for r in range(1, rep):
                q_g = jnp.where(row_id % rep == r, q[:, r * d_head:(r + 1) * d_head], q_g)
            qs.append(q_g.astype(dtype))

        sums = []
        for g in range(n_kv):
            wait_for(("k", g), k_ref.at[g])
            start_until(started + _STEP)
            s = lax.dot_general(qs[g], k_ref[g], (((1,), (1,)), ((), ())),
                                preferred_element_type=_F32)
            s = rnd(rnd(s) * scale)
            p = jnp.exp(s - jnp.max(s, axis=-1, keepdims=True))
            sums.append(jnp.sum(p, axis=-1, keepdims=True))
            p_ref[g] = p

        heads = []
        for g in range(n_kv):
            wait_for(("v", g), v_ref.at[g])
            start_until(started + _STEP // 2)
            o = jnp.dot(p_ref[g].astype(dtype), v_ref[g], preferred_element_type=_F32) / sums[g]
            heads += [jnp.where(row_id == r, o, 0.0) for r in range(rep)]

        wait_for("wo", wo_ref)
        start_until(len(issue))
        attn = jnp.dot(jnp.concatenate(heads, axis=1).astype(dtype), wo_ref[...],
                       preferred_element_type=_F32)
        h = rnd(x + rnd(jnp.sum(attn, axis=0, keepdims=True)))
        y = layernorm(layernorm(h)).astype(dtype)

        wait_for("w1", w1_ref)
        z = jnp.dot(y, w1_ref[...], preferred_element_type=_F32)
        z = z + b1_ref[...].astype(_F32).reshape(1, d_ff)
        act = rnd(jax.nn.gelu(z, approximate=True))

        for c in range(0, d_ff, _LANES):
            act_ref[pl.ds(c, _LANES), :] = jnp.broadcast_to(
                act[:1, c:c + _LANES], (_LANES, _LANES)).T
        res = h + b2_ref[...].astype(_F32).reshape(1, d_model)
        cols = range(0, d_model, _LANES)
        acc = [jnp.where(row_id == 0, res[:, c:c + _LANES], 0.0) for c in cols]
        for g in range(len(_W2_GROUPS) + 1):
            mine = [c for c in run if c[2] == ("w2", g)]
            for c in mine:
                copy(c).wait()
            for _, (row, rows, col, _), _, _ in mine:
                if col > 0:
                    continue
                for r in range(row, row + rows, _ROWS):
                    a = act_ref[pl.ds(r, _ROWS), :]
                    w = w2_ref[pl.ds(r, _ROWS), :].astype(_F32)
                    acc = [t + a * w[:, c:c + _LANES] for t, c in zip(acc, cols)]
        out_ref[0] = jnp.sum(jnp.concatenate(acc, axis=1), axis=0, keepdims=True).astype(dtype)

        done = pltpu.make_async_copy(out_ref, out_hbm, io_sem)
        done.start()
        done.wait()

    hbm = pl.BlockSpec(memory_space=pltpu.MemorySpace.HBM)
    return pl.pallas_call(
        kernel,
        in_specs=[hbm] * 9,
        out_specs=hbm,
        out_shape=jax.ShapeDtypeStruct(A_x.shape, dtype),
        scratch_shapes=[
            pltpu.VMEM(A_x.shape, dtype),
            pltpu.VMEM((n_kv, window, d_head), dtype),
            pltpu.VMEM((n_kv, window, d_head), dtype),
            pltpu.VMEM(A_wq.shape, dtype),
            pltpu.VMEM(A_wo.shape, dtype),
            pltpu.VMEM(B_w1.shape, dtype),
            pltpu.VMEM(B_b1.shape, dtype),
            pltpu.VMEM(B_w2.shape, dtype),
            pltpu.VMEM(B_b2.shape, dtype),
            pltpu.VMEM(A_x.shape, dtype),
            pltpu.VMEM((n_kv, _ROWS, window), _F32),
            pltpu.VMEM((d_ff, _LANES), _F32),
            pltpu.SemaphoreType.DMA((len(sem_of),)),
            pltpu.SemaphoreType.DMA(()),
        ],
        compiler_params=pltpu.CompilerParams(
            vmem_limit_bytes=64 * 2**20,
            disable_bounds_checks=True,
            disable_semaphore_checks=True,
        ),
    )(A_x, A_k_cache, A_v_cache, A_wq, A_wo, B_w1, B_b1, B_w2, B_b2)
```

```python
import jax
import jax.numpy as jnp
import numpy as np
from jax import lax
import jax.experimental.pallas as pl
import jax.experimental.pallas.tpu as pltpu

_F32 = jnp.float32
_EPS = 1e-5
_LANES = 128
_ROWS = 8

_PIECE = 16
_ROUNDS = 8
_FIRST_TILE = {"wq": 16, "wo": 16, "w1": 16, "w2": 24}
_W2_EARLY = 10
_LEAD = 27
_TAIL_PIECES = 4
_TAIL_TILES = 2
_AHEAD = 80
_WO_PARTS = 4
_W2_GROUPS = (16, 8, 8, 4, 2, 1, 1)


def _rects(shape, lo, hi):
    per_row = shape[1] // _LANES
    out = []
    while lo < hi:
        r, c = divmod(lo, per_row)
        if c == 0 and hi - lo >= per_row:
            n = (hi - lo) // per_row
            out.append((r * _ROWS, n * _ROWS, 0, shape[1]))
            lo += n * per_row
        else:
            n = min(per_row - c, hi - lo)
            out.append((r * _ROWS, _ROWS, c * _LANES, n * _LANES))
            lo += n
    return out


def _num_tiles(shape):
    return shape[0] // _ROWS * (shape[1] // _LANES)


def _rounds(names, shapes):
    rounds = [[] for _ in range(_ROUNDS)]
    for name in names:
        first, tiles = _FIRST_TILE.get(name, 0), _num_tiles(shapes[name])
        assert tiles % (2 * _PIECE) == 0
        for b, lo in enumerate(range(first, first + tiles, 2 * _PIECE)):
            rounds[b % _ROUNDS].append((name, lo))
    return rounds


def _pieces(rounds):
    return [(name, lo + t) for blocks in rounds for t in (0, _PIECE) for name, lo in blocks]


def _in_pairs(blocks):
    return [blocks[i:i + 2] for i in range(0, len(blocks), 2)]


def _plan(shapes, k_names, v_names):
    wq, wo, w1, w2 = (sum(_rounds([n], shapes), []) for n in ("wq", "wo", "w1", "w2"))
    mlp = []
    for i, block in enumerate(w1):
        mlp += [block] + w2[i * _W2_EARLY // len(w1):(i + 1) * _W2_EARLY // len(w1)]
    mlp += w2[_W2_EARLY:]
    pieces = _pieces(_in_pairs(wq) + _rounds(k_names, shapes) + _rounds(v_names, shapes)
                     + _in_pairs(wo) + _in_pairs(mlp))

    w2_group = [g + 1 for g, n in enumerate(_W2_GROUPS) for _ in range(n)]
    w2_group = [0] * (len(pieces) - len(w2_group)) + w2_group
    run = []
    for i, (name, lo) in enumerate(pieces):
        tiles = _num_tiles(shapes[name])
        group = name
        if name == "w2":
            assert lo % (shapes[name][1] // _LANES) == 0
            group = (name, w2_group[i])
        elif name == "wo":
            assert lo % _PIECE == 0
            group = (name, lo % tiles * _WO_PARTS // tiles)
        tail = i >= len(pieces) - _TAIL_PIECES
        size = _TAIL_TILES if tail else _PIECE
        for t in range(lo, lo + _PIECE, size):
            rects = (_rects(shapes[name], min(t, tiles), min(t + size, tiles))
                     + _rects(shapes[name], max(t - tiles, 0), max(t + size - tiles, 0)))
            run += [(name, rect, group, 1 if tail else 1 - i % 2) for rect in rects]

    low = [c for c in run if c[3] == 1]
    issue, rest = low[:_LEAD], low[_LEAD:][::-1]
    for c in run:
        if c[3] == 0:
            issue.append(c)
        elif rest:
            issue.append(rest.pop())
    return run, issue


@jax.jit
def pallas_sequential_preLN__sliding_block_cached__mixer_channel_mlp__decode_kernel(
    A_x: jax.Array,
    A_k_cache: jax.Array,
    A_v_cache: jax.Array,
    A_wq: jax.Array,
    A_wo: jax.Array,
    B_x: jax.Array,
    B_w1: jax.Array,
    B_b1: jax.Array,
    B_w2: jax.Array,
    B_b2: jax.Array,
):
    del B_x
    dtype = A_x.dtype
    d_model, d_ff = B_w1.shape
    _, n_kv, seq, d_head = A_k_cache.shape
    rep = A_wq.shape[1] // d_head // n_kv
    window = min(4096, max(256, seq // 4))
    assert A_x.shape == (1, 1, d_model) and d_head == _LANES and _ROWS % rep == 0
    scale = float(np.float32(d_head ** -0.5).astype(dtype))

    k_names = [("k", g) for g in range(n_kv)]
    v_names = [("v", g) for g in range(n_kv)]
    shapes = {"wq": A_wq.shape, "wo": A_wo.shape, "w1": B_w1.shape, "w2": B_w2.shape}
    shapes.update({name: (window, d_head) for name in k_names + v_names})
    run, issue = _plan(shapes, k_names, v_names)
    sem_of, due = {}, {}
    for n, c in enumerate(run):
        sem_of.setdefault(c[2], len(sem_of))
        due[c[2]] = n + _AHEAD
    for n, c in enumerate(issue):
        due[c[2]] = max(due[c[2]], n + 1)

    def rnd(a):
        return a.astype(dtype).astype(_F32)

    def layernorm(a):
        mean = jnp.mean(a, axis=-1, keepdims=True)
        var = jnp.mean(jnp.square(a - mean), axis=-1, keepdims=True)
        return rnd(rnd(a - rnd(mean)) / rnd(jnp.sqrt(rnd(rnd(var) + _EPS))))

    def kernel(x_hbm, k_hbm, v_hbm, wq_hbm, wo_hbm, w1_hbm, b1_hbm, w2_hbm, b2_hbm, out_ref,
               x_ref, k_ref, v_ref, wq_ref, wo_ref, w1_ref, b1_ref, w2_ref, b2_ref,
               p_ref, act_ref, sems, vector_sems):
        refs = {"k": (k_hbm, k_ref), "v": (v_hbm, v_ref), "wq": (wq_hbm, wq_ref),
                "wo": (wo_hbm, wo_ref), "w1": (w1_hbm, w1_ref), "w2": (w2_hbm, w2_ref)}

        def copy(c):
            name, (row, rows, col, cols), group, _ = c
            if isinstance(name, tuple):
                src, dst = refs[name[0]]
                src = src.at[0, name[1], pl.ds(seq - window + row, rows), :]
                dst = dst.at[name[1], pl.ds(row, rows), :]
            else:
                src, dst = (r.at[pl.ds(row, rows), pl.ds(col, cols)] for r in refs[name])
            return pltpu.make_async_copy(src, dst, sems.at[sem_of[group]])

        started = 0

        def start_until(n):
            nonlocal started
            for c in issue[started:n]:
                copy(c).start(priority=c[3])
            started = max(started, min(n, len(issue)))

        def wait_for(group, buf, refill=0):
            start_until(due[group])
            pltpu.make_async_copy(buf, buf, sems.at[sem_of[group]]).wait()
            start_until(started + refill)

        start_until(_LEAD)
        vectors = [pltpu.make_async_copy(src, dst, vector_sems.at[i]) for i, (src, dst) in
                   enumerate(((x_hbm, x_ref), (b1_hbm, b1_ref), (b2_hbm, b2_ref)))]
        for c in vectors:
            c.start()
        start_until(_LEAD + _AHEAD)
        for c in vectors:
            c.wait()

        x = jnp.broadcast_to(x_ref[0].astype(_F32), (_ROWS, d_model))
        xn = layernorm(x).astype(dtype)
        row_id = lax.broadcasted_iota(jnp.int32, (_ROWS, _LANES), 0)

        wait_for("wq", wq_ref)
        qs = []
        for g in range(n_kv):
            q = jnp.dot(xn, wq_ref[:, pl.ds(g * rep * d_head, rep * d_head)],
                        preferred_element_type=_F32)
            q_g = q[:, :d_head]
            for r in range(1, rep):
                q_g = jnp.where(row_id % rep == r, q[:, r * d_head:(r + 1) * d_head], q_g)
            qs.append(q_g.astype(dtype))

        sums = []
        for g in range(n_kv):
            wait_for(("k", g), k_ref.at[g], refill=16)
            s = lax.dot_general(qs[g], k_ref[g], (((1,), (1,)), ((), ())),
                                preferred_element_type=_F32)
            s = rnd(rnd(s) * scale)
            p = jnp.exp(s - jnp.max(s, axis=-1, keepdims=True))
            sums.append(jnp.sum(p, axis=-1, keepdims=True))
            p_ref[g] = p

        heads = []
        for g in range(n_kv):
            wait_for(("v", g), v_ref.at[g], refill=8)
            o = jnp.dot(p_ref[g].astype(dtype), v_ref[g], preferred_element_type=_F32) / sums[g]
            heads += [jnp.where(row_id == r, o, 0.0) for r in range(rep)]

        attn = jnp.zeros((_ROWS, d_model), _F32)
        per_part = len(heads) // _WO_PARTS
        for t in range(_WO_PARTS):
            rows = pl.ds(t * per_part * d_head, per_part * d_head)
            wait_for(("wo", t), wo_ref.at[rows], refill=12)
            o = jnp.concatenate(heads[t * per_part:(t + 1) * per_part], axis=1)
            attn += jnp.dot(o.astype(dtype), wo_ref[rows, :], preferred_element_type=_F32)
        start_until(len(issue))
        h = rnd(x + rnd(jnp.sum(attn, axis=0, keepdims=True)))
        y = layernorm(layernorm(h)).astype(dtype)

        wait_for("w1", w1_ref)
        z = jnp.dot(y, w1_ref[...], preferred_element_type=_F32)
        z = z + b1_ref[...].astype(_F32).reshape(1, d_ff)
        act = rnd(jax.nn.gelu(z, approximate=True))

        for c in range(0, d_ff, _LANES):
            act_ref[pl.ds(c, _LANES), :] = jnp.broadcast_to(
                act[:1, c:c + _LANES], (_LANES, _LANES)).T
        res = h + b2_ref[...].astype(_F32).reshape(1, d_model)
        cols = range(0, d_model, _LANES)
        acc = [jnp.where(row_id == 0, res[:, c:c + _LANES], 0.0) for c in cols]
        for g in range(len(_W2_GROUPS) + 1):
            mine = [c for c in run if c[2] == ("w2", g)]
            for c in mine:
                copy(c).wait()
            for _, (row, rows, col, _), _, _ in mine:
                if col > 0:
                    continue
                for r in range(row, row + rows, _ROWS):
                    a = act_ref[pl.ds(r, _ROWS), :]
                    w = w2_ref[pl.ds(r, _ROWS), :].astype(_F32)
                    acc = [t + a * w[:, c:c + _LANES] for t, c in zip(acc, cols)]
        out_ref[0] = jnp.sum(jnp.concatenate(acc, axis=1), axis=0, keepdims=True).astype(dtype)

    return pl.pallas_call(
        kernel,
        in_specs=[pl.BlockSpec(memory_space=pltpu.MemorySpace.HBM)] * 9,
        out_specs=pl.BlockSpec(memory_space=pltpu.MemorySpace.VMEM),
        out_shape=jax.ShapeDtypeStruct(A_x.shape, dtype),
        scratch_shapes=[
            pltpu.VMEM(A_x.shape, dtype),
            pltpu.VMEM((n_kv, window, d_head), dtype),
            pltpu.VMEM((n_kv, window, d_head), dtype),
            pltpu.VMEM(A_wq.shape, dtype),
            pltpu.VMEM(A_wo.shape, dtype),
            pltpu.VMEM(B_w1.shape, dtype),
            pltpu.VMEM(B_b1.shape, dtype),
            pltpu.VMEM(B_w2.shape, dtype),
            pltpu.VMEM(B_b2.shape, dtype),
            pltpu.VMEM((n_kv, _ROWS, window), _F32),
            pltpu.VMEM((d_ff, _LANES), _F32),
            pltpu.SemaphoreType.DMA((len(sem_of),)),
            pltpu.SemaphoreType.DMA((3,)),
        ],
        compiler_params=pltpu.CompilerParams(
            vmem_limit_bytes=64 * 2**20,
            disable_semaphore_checks=True,
        ),
    )(A_x, A_k_cache, A_v_cache, A_wq, A_wo, B_w1, B_b1, B_w2, B_b2)
```
